```python
import os as _os
_os.environ.setdefault("JAX_PLATFORMS", "cpu")
import jax
import jax.numpy as jnp

def _softmax(x, axis=-1):
    return jax.nn.softmax(x, axis=axis)
def _gelu(x):
    return jax.nn.gelu(x, approximate=True)
def _silu(x):
    return jax.nn.silu(x)
def _sigmoid(x):
    return jax.nn.sigmoid(x)
def _layernorm(x, axis=-1, eps=1e-5):
    m = jnp.mean(x, axis=axis, keepdims=True)
    v = jnp.var(x, axis=axis, keepdims=True)
    return (x - m) / jnp.sqrt(v + eps)
def _scatter_add(tgt, idx, src, axis=0):
    return tgt.at[idx].add(src)
def _segment_sum(src, seg, n):
    return jax.ops.segment_sum(src, seg, n)
class _Rng:
    def __init__(self, key):
        self._k = key
    def _next(self):
        self._k, sub = jax.random.split(self._k)
        return sub
    def normal(self, shape):
        return jax.random.normal(self._next(), shape, dtype=jnp.bfloat16)
    def randint(self, lo, hi, shape):
        return jax.random.randint(self._next(), shape, lo, hi, dtype=jnp.int32)
    def uniform(self, shape, lo=0.0, hi=1.0):
        return jax.random.uniform(self._next(), shape, jnp.bfloat16, lo, hi)
    def permutation(self, n):
        return jax.random.permutation(self._next(), n)


kernel_name = 'interleave_layers__gqa_block_cached__dense_activation_silu__decode'

def setup_inputs():
    _rng = _Rng(jax.random.key(int.from_bytes(__import__("os").urandom(4), "little")))
    _w = (lambda a: (lambda t: t.astype(jnp.bfloat16) if jnp.issubdtype(t.dtype, jnp.floating) else t)(jnp.asarray(a)))
    def _A_setup():
        B, Sq, D = 2, 1, 512
        Hq, Hkv, Sk, Dh = 32, 8, 8192, 128
        assert Hq % Hkv == 0, (Hq, Hkv)
        return {
            "x": _w((lambda *s: _rng.normal(s) * 0.1)(B, Sq, D)),
            "k_cache": _w((lambda *s: _rng.normal(s) * 0.8)(B, Hkv, Sk, Dh)),
            "v_cache": _w((lambda *s: _rng.normal(s) * 1.6)(B, Hkv, Sk, Dh)),
            "wq": _w((lambda *s: _rng.normal(s) * 0.8)(D, Hq * Dh) * (D ** -0.5)),
            "wo": _w((lambda *s: _rng.normal(s) * 1.6)(Hq * Dh, D) * ((Hq * Dh) ** -0.5)),
        }
    _A_in = _A_setup()

    def _B_setup():
        B, S, D, F = 2, 1, 512, 1792
        return {
            "x": _w((lambda *s: _rng.normal(s) * 0.1)(B, S, D)),
            "w1": _w((lambda *s: _rng.normal(s) * 0.4)(D, F) * (D ** -0.5)),
            "w2": _w((lambda *s: _rng.normal(s) * 0.4)(F, D) * (F ** -0.5)),
        }
    _B_in = _B_setup()

    return {
        "A_x": _A_in["x"],
        "A_k_cache": _A_in["k_cache"],
        "A_v_cache": _A_in["v_cache"],
        "A_wq": _A_in["wq"],
        "A_wo": _A_in["wo"],
        "B_x": _B_in["x"],
        "B_w1": _B_in["w1"],
        "B_w2": _B_in["w2"],
    }

def reference(A_x, A_k_cache, A_v_cache, A_wq, A_wo, B_x, B_w1, B_w2):
    def _A_ref(x, k_cache, v_cache, wq, wo):
        B, Sq, D = x.shape
        Hq, Dh = 32, 128
        Hkv = k_cache.shape[1]
        rep = Hq // Hkv
        q = (lambda x, *d: x.transpose(*d))((x @ wq).reshape(B, Sq, Hq, Dh), 0, 2, 1, 3)
        k = jnp.repeat(k_cache, rep, axis=1)
        v = jnp.repeat(v_cache, rep, axis=1)
        scores = jnp.einsum("bhqd,bhkd->bhqk", q, k) * (Dh ** -0.5)
        p = _softmax(scores, axis=-1)
        o = jnp.einsum("bhqk,bhkd->bhqd", p, v)
        return (lambda x, *d: x.transpose(*d))(o, 0, 2, 1, 3).reshape(B, Sq, Hq * Dh) @ wo

    def _B_ref(x, w1, w2):
        h = jnp.einsum("bsd,df->bsf", x, w1)
        h = _silu(h)
        out = jnp.einsum("bsf,fd->bsd", h, w2)
        return out

    x = A_x
    x = x + _A_ref(_layernorm(x, axis=-1), A_k_cache, A_v_cache, A_wq, A_wo)
    x = x + _B_ref(_layernorm(x, axis=-1), B_w1, B_w2)
    x = x + _A_ref(_layernorm(x, axis=-1), A_k_cache, A_v_cache, A_wq, A_wo)
    x = x + _B_ref(_layernorm(x, axis=-1), B_w1, B_w2)
    return x
```

```python
import jax
import jax.numpy as jnp
import jax.experimental.pallas as pl
import jax.experimental.pallas.tpu as pltpu

_T = 128
_R = 8
_CH = 2048


def _layernorm(x):
    m = jnp.mean(x, axis=-1, keepdims=True)
    c = x - m
    v = jnp.mean(c * c, axis=-1, keepdims=True)
    return c / jnp.sqrt(v + 1e-5)


@jax.jit
def pallas_interleave_layers__gqa_block_cached__dense_activation_silu__decode_kernel(
    A_x: jax.Array,
    A_k_cache: jax.Array,
    A_v_cache: jax.Array,
    A_wq: jax.Array,
    A_wo: jax.Array,
    B_x: jax.Array,
    B_w1: jax.Array,
    B_w2: jax.Array,
):
    del B_x
    B, Sq, D = A_x.shape
    _, Hkv, Sk, Dh = A_k_cache.shape
    HD = A_wq.shape[1]
    Hq = HD // Dh
    F = B_w1.shape[1]
    rep = Hq // Hkv
    assert Sq == 1 and Dh == _T and _R % rep == 0 and Hq % _R == 0
    per = _R // rep
    G = Hq // _R
    NT = Sk // _T
    NC = Sk // _CH
    scale = float(Dh) ** -0.5
    f32, bf16 = jnp.float32, jnp.bfloat16

    def kernel(x_ref, k_hbm, v_hbm, wq_hbm, wo_hbm, w1_hbm, w2_hbm, o_ref,
               kb, vb, wqb, wob, w1b, w2b, q_scr, a_scr, ksem, vsem, wsem):
        def kv_chunk(src, dst, sem, b, h, c):
            r = pl.ds(c * _CH, _CH)
            return pltpu.make_async_copy(src.at[b, h, r], dst.at[b, h, r], sem.at[b * Hkv + h])

        def kv_all(src, dst, sem, b, h):
            return pltpu.make_async_copy(src.at[b, h], dst.at[b, h], sem.at[b * Hkv + h])

        w_copies = [pltpu.make_async_copy(s, d, wsem.at[i]) for i, (s, d) in enumerate(
            ((wq_hbm, wqb), (wo_hbm, wob), (w1_hbm, w1b), (w2_hbm, w2b)))]

        w_copies[0].start()
        for b in range(B):
            for h in range(Hkv):
                for c in range(NC):
                    kv_chunk(k_hbm, kb, ksem, b, h, c).start()
                for c in range(NC):
                    kv_chunk(v_hbm, vb, vsem, b, h, c).start()
            if b == 0:
                for w in w_copies[1:]:
                    w.start()

        row = jax.lax.broadcasted_iota(jnp.int32, (_R, _T), 0)

        def q_proj(x):
            xn = _layernorm(x).astype(bf16)
            for g in range(G):
                q = jnp.zeros((_R, _T), f32)
                for r in range(_R):
                    j = g * _R + r
                    qj = jnp.dot(xn, wqb[:, j * _T:(j + 1) * _T], preferred_element_type=f32)
                    q = jnp.where(row == r, qj, q)
                q_scr[g] = q
                a_scr[g] = jnp.zeros((_R, _T), f32)

        def attend(b, h, first):
            g = h // per
            q = q_scr[g].astype(bf16)
            if first:
                kv_all(k_hbm, kb, ksem, b, h).wait()
            ss = []
            for j in range(NT):
                t = pl.ds(j * _T, _T)
                kt = kb[b, h, t, :]
                if first:
                    kt = kt.T
                    kb[b, h, t, :] = kt
                ss.append(jnp.dot(q, kt, preferred_element_type=f32) * scale)
            m = ss[0]
            for s in ss[1:]:
                m = jnp.maximum(m, s)
            m = jnp.max(m, axis=-1, keepdims=True)
            if first:
                kv_all(v_hbm, vb, vsem, b, h).wait()
            l = jnp.zeros((_R, _T), f32)
            acc = jnp.zeros((_R, _T), f32)
            for j in range(NT):
                p = jnp.exp(ss[j] - m)
                l = l + p
                acc = acc + jnp.dot(p.astype(bf16), vb[b, h, pl.ds(j * _T, _T), :],
                                    preferred_element_type=f32)
            o = acc / jnp.sum(l, axis=-1, keepdims=True)
            a_scr[g] = jnp.where(row // rep == h % per, o, a_scr[g])

        def o_proj():
            acc = jnp.zeros((_R, D), f32)
            for g in range(G):
                a = a_scr[g]
                for r in range(_R):
                    j = g * _R + r
                    aj = jnp.where(row == r, a, 0.0).astype(bf16)
                    acc = acc + jnp.dot(aj, wob[j * _T:(j + 1) * _T, :], preferred_element_type=f32)
            return jnp.broadcast_to(jnp.sum(acc, axis=0, keepdims=True), (_R, D))

        def ffn(x):
            xn = _layernorm(x).astype(bf16)
            hid = jnp.dot(xn, w1b[...], preferred_element_type=f32)
            hid = hid * jax.nn.sigmoid(hid)
            return jnp.dot(hid.astype(bf16), w2b[...], preferred_element_type=f32)

        def per_batch(b, carry):
            x = jnp.broadcast_to(x_ref[b].astype(f32), (_R, D))

            @pl.when(b == 0)
            def _():
                w_copies[0].wait()

            q_proj(x)
            jax.lax.fori_loop(0, Hkv, lambda h, c: (attend(b, h, True), c)[1], 0)

            @pl.when(b == 0)
            def _():
                for w in w_copies[1:]:
                    w.wait()

            x = x + o_proj()
            x = x + ffn(x)
            q_proj(x)
            jax.lax.fori_loop(0, Hkv, lambda h, c: (attend(b, h, False), c)[1], 0)
            x = x + o_proj()
            x = x + ffn(x)
            o_ref[b] = x[0:1, :].astype(o_ref.dtype)
            return carry

        jax.lax.fori_loop(0, B, per_batch, 0)

    any_spec = pl.BlockSpec(memory_space=pl.ANY)
    vmem_spec = pl.BlockSpec(memory_space=pltpu.VMEM)
    return pl.pallas_call(
        kernel,
        out_shape=jax.ShapeDtypeStruct((B, Sq, D), A_x.dtype),
        in_specs=[vmem_spec] + [any_spec] * 6,
        out_specs=vmem_spec,
        scratch_shapes=[
            pltpu.VMEM(A_k_cache.shape, bf16),
            pltpu.VMEM(A_v_cache.shape, bf16),
            pltpu.VMEM(A_wq.shape, bf16),
            pltpu.VMEM(A_wo.shape, bf16),
            pltpu.VMEM(B_w1.shape, bf16),
            pltpu.VMEM(B_w2.shape, bf16),
            pltpu.VMEM((G, _R, _T), f32),
            pltpu.VMEM((G, _R, _T), f32),
            pltpu.SemaphoreType.DMA((B * Hkv,)),
            pltpu.SemaphoreType.DMA((B * Hkv,)),
            pltpu.SemaphoreType.DMA((4,)),
        ],
        compiler_params=pltpu.CompilerParams(vmem_limit_bytes=100 * 1024 * 1024),
    )(A_x, A_k_cache, A_v_cache, A_wq, A_wo, B_w1, B_w2)
```

```python
import jax
import jax.numpy as jnp
import jax.experimental.pallas as pl
import jax.experimental.pallas.tpu as pltpu

_T = 128
_R = 8
_CH = 2048
_AHEAD = 3
_TAIL = 1024


def _center(x):
    c = x - jnp.mean(x, axis=-1, keepdims=True)
    r = 1.0 / jnp.sqrt(jnp.mean(c * c, axis=-1, keepdims=True) + 1e-5)
    return c, r


@jax.jit
def pallas_interleave_layers__gqa_block_cached__dense_activation_silu__decode_kernel(
    A_x: jax.Array,
    A_k_cache: jax.Array,
    A_v_cache: jax.Array,
    A_wq: jax.Array,
    A_wo: jax.Array,
    B_x: jax.Array,
    B_w1: jax.Array,
    B_w2: jax.Array,
):
    del B_x
    B, Sq, D = A_x.shape
    _, Hkv, Sk, Dh = A_k_cache.shape
    HD = A_wq.shape[1]
    Hq = HD // Dh
    F = B_w1.shape[1]
    rep = Hq // Hkv
    assert Sq == 1 and Dh == _T and _R % rep == 0 and Hq % _R == 0 and B <= _R
    per = _R // rep
    NT = Sk // _T
    scale = float(Dh) ** -0.5
    f32, bf16, u32 = jnp.float32, jnp.bfloat16, jnp.uint32

    def mm(a, b):
        return jnp.dot(a, b, preferred_element_type=f32)

    def kernel(x_hbm, k_hbm, v_hbm, wq_hbm, wo_hbm, w1_hbm, w2_hbm, ob,
               kb, vb, wqb, wob, w1b, w2b, xb, a_scr, s_scr, p_scr,
               ksem, vsem, wsem):
        def rows(src, dst, sem, b, h, lo, hi):
            r = pl.ds(lo, hi - lo)
            return pltpu.make_async_copy(src.at[b, h, r], dst.at[b, h, r], sem)

        def k_rows(n, lo, hi):
            return rows(k_hbm, kb, ksem.at[n % _AHEAD], n // Hkv, n % Hkv, lo, hi)

        def v_rows(n, lo, hi, sem=None):
            sem = vsem.at[n % _AHEAD] if sem is None else sem
            return rows(v_hbm, vb, sem, n // Hkv, n % Hkv, lo, hi)

        def start_rows(fn, n, lo, hi, step, **kw):
            for r in range(lo, hi, step):
                fn(n, r, min(r + step, hi), **kw).start()

        x_cp = pltpu.make_async_copy(x_hbm, xb, wsem.at[0])
        wq_cp, wo_cp, w1_cp, w2_cp = [
            pltpu.make_async_copy(s.bitcast(u32), d, wsem.at[i]) for s, d, i in
            ((wq_hbm, wqb, 0), (wo_hbm, wob, 1), (w1_hbm, w1b, 0), (w2_hbm, w2b, 0))]
        last = B * Hkv - 1
        cuts = (Sk - 2 * _TAIL, Sk - _TAIL, Sk)

        x_cp.start()
        wq_cp.start()

        row = jax.lax.broadcasted_iota(jnp.int32, (_R, _T), 0)
        zeros = jnp.zeros((_R, _T), f32)

        def tile(j):
            return pl.ds(pl.multiple_of(j * _T, _T), _T)

        kw = kb.bitcast(jnp.uint32)
        vw = vb.bitcast(jnp.uint32)

        def ld(w, b, h, j):
            return pltpu.bitcast(w[b, h, pl.ds(j * (_T // 2), _T // 2), :], bf16)

        def wt(w, i, j):
            return pltpu.bitcast(w[pl.ds(pl.multiple_of(i * (_T // 2), _T // 2), _T // 2), tile(j)], bf16)

        def split(x):
            return [x[:, i * _T:(i + 1) * _T].astype(bf16) for i in range(x.shape[1] // _T)]

        def col(xs, w, j):
            y = None
            for i, xi in enumerate(xs):
                t = mm(xi, wt(w, i, j))
                y = t if y is None else y + t
            return y

        def q_head(xs, r, h):
            q = zeros
            for i in range(rep):
                q = jnp.where(row == (h % per) * rep + i, col(xs, wqb, h * rep + i), q)
            return (q * r).astype(bf16)

        def o_head(acc, a, h):
            for r in range(rep):
                ar = jnp.where(row == (h % per) * rep + r, a, 0.0).astype(bf16)
                acc = tuple(c + mm(ar, wt(wob, h * rep + r, j)) for j, c in enumerate(acc))
            return acc

        def fold(acc):
            acc = jnp.concatenate(acc, axis=1)
            return jnp.broadcast_to(jnp.sum(acc, axis=0, keepdims=True), (_R, D))

        def ffn(x):
            c, r = _center(x)
            xn = split(c)
            hs = []
            for j in range(F // _T):
                hid = col(xn, w1b, j) * r
                hs.append((hid * jax.nn.sigmoid(hid)).astype(bf16))
            return x + jnp.concatenate([col(hs, w2b, j) for j in range(D // _T)], axis=1)

        def first_pass_head(b, xs, r, h, acc):
            n = b * Hkv + h
            q = q_head(xs, r, h)
            k_rows(n, 0, Sk).wait()

            @pl.when(n + _AHEAD == Hkv)
            def _():
                w1_cp.start()
                w2_cp.start()

            @pl.when(n + _AHEAD <= last)
            def _():
                start_rows(k_rows, n + _AHEAD, 0, Sk, _CH)

            m = None
            for j in range(NT):
                kt = ld(kw, b, h, j).T
                kw[b, h, pl.ds(j * (_T // 2), _T // 2), :] = pltpu.bitcast(kt, jnp.uint32)
                s = mm(q, kt) * scale
                s_scr[0, j] = s
                m = s if m is None else jnp.maximum(m, s)
            m = jnp.max(m, axis=-1, keepdims=True)
            l = zeros
            for j in range(NT):
                p = jnp.exp(s_scr[0, j] - m)
                l = l + p
                p_scr[0, j] = p
            inv = 1.0 / jnp.sum(l, axis=-1, keepdims=True)

            @pl.when(n == 0)
            def _():
                wo_cp.wait()

            @pl.when(n < last)
            def _():
                v_rows(n, 0, Sk).wait()

            @pl.when(n == last)
            def _():
                v_rows(n, 0, cuts[0]).wait()

            @pl.when(n + _AHEAD < last)
            def _():
                start_rows(v_rows, n + _AHEAD, 0, Sk, _CH)

            @pl.when(n + _AHEAD == last)
            def _():
                start_rows(v_rows, last, 0, cuts[0] - _CH, _CH)
                start_rows(v_rows, last, cuts[0] - _CH, cuts[0], _CH // 2)
                for i in range(2):
                    start_rows(v_rows, last, cuts[i], cuts[i + 1], _TAIL // 2, sem=wsem.at[i])

            o = zeros
            for i, (lo, hi) in enumerate(zip((0,) + cuts, cuts)):
                if i:
                    @pl.when(n == last)
                    def _():
                        v_rows(n, lo, hi, sem=wsem.at[i - 1]).wait()
                for j in range(lo // _T, hi // _T):
                    o = o + mm(p_scr[0, j].astype(bf16), ld(vw, b, h, j))
            return o_head(acc, o * inv, h)

        def qk_tile(b, h, q, slot, j, m):
            s = mm(q, ld(kw, b, h, j)) * scale
            s_scr[slot, j] = s
            return s if m is None else jnp.maximum(m, s)

        def exp_tile(slot, j, m, l):
            p = jnp.exp(s_scr[slot, j] - m)
            p_scr[slot, j] = p
            return l + p

        def pv_all(b, h):
            o = zeros
            for j in range(NT):
                o = o + mm(p_scr[h % 2, j].astype(bf16), ld(vw, b, h, j))
            return o

        def rowmax(m):
            return jnp.broadcast_to(jnp.max(m, axis=-1, keepdims=True), (_R, _T))

        def second_pass_step(b, h, m, q):
            mn, l, o = None, zeros, zeros
            for j in range(NT):
                mn = qk_tile(b, h + 1, q, (h + 1) % 2, j, mn)
                l = exp_tile(h % 2, j, m, l)
            o = pv_all(b, h)
            a_scr[h] = o / jnp.sum(l, axis=-1, keepdims=True)
            return rowmax(mn)

        def first_pass(b, x):
            c, r = _center(x)
            xs = split(c)
            return jax.lax.fori_loop(0, Hkv, lambda h, a: first_pass_head(b, xs, r, h, a),
                                     (zeros,) * (D // _T))

        def second_pass(b, x):
            c, r = _center(x)
            xs = split(c)
            qs = [q_head(xs, r, h) for h in range(Hkv)]
            m = None
            for j in range(NT):
                m = qk_tile(b, 0, qs[0], 0, j, m)
            m = rowmax(m)
            for h in range(Hkv - 2):
                m = second_pass_step(b, h, m, qs[h + 1])
            h = Hkv - 2
            mn, l = None, zeros
            for j in range(NT):
                mn = qk_tile(b, h + 1, qs[h + 1], (h + 1) % 2, j, mn)
                l = exp_tile(h % 2, j, m, l)
            m = rowmax(mn)
            l2, o = zeros, zeros
            for j in range(NT):
                o = o + mm(p_scr[h % 2, j].astype(bf16), ld(vw, b, h, j))
                l2 = exp_tile((h + 1) % 2, j, m, l2)
            a_scr[h] = o / jnp.sum(l, axis=-1, keepdims=True)
            o = pv_all(b, h + 1)
            acc = (zeros,) * (D // _T)
            for hh in range(Hkv - 1):
                acc = o_head(acc, a_scr[hh], hh)
            return o_head(acc, o / jnp.sum(l2, axis=-1, keepdims=True), h + 1)

        def layer_pair(i, x):
            b = i // 2
            first = i % 2 == 0

            @pl.when(i == 0)
            def _():
                wo_cp.start()
                x_cp.wait()
                wq_cp.wait()
                for n in range(_AHEAD):
                    start_rows(k_rows, n, 0, Sk, _CH)
                    start_rows(v_rows, n, 0, Sk, _CH)

            xin = xb[...].astype(f32)
            x0 = jnp.broadcast_to(xin[0:1], (_R, D))
            for bb in range(1, B):
                x0 = jnp.where(b == bb, jnp.broadcast_to(xin[bb:bb + 1], (_R, D)), x0)
            x = jnp.where(first, x0, x)

            acc = jax.lax.cond(first, lambda: first_pass(b, x), lambda: second_pass(b, x))

            @pl.when(i == 0)
            def _():
                w1_cp.wait()
                w2_cp.wait()

            x = ffn(x + fold(acc))
            ob[b] = x[0:1].astype(ob.dtype)
            return x

        jax.lax.fori_loop(0, 2 * B, layer_pair, jnp.zeros((_R, D), f32))

    any_spec = pl.BlockSpec(memory_space=pl.ANY)
    out = pl.pallas_call(
        kernel,
        out_shape=jax.ShapeDtypeStruct((B, Sq, D), A_x.dtype),
        in_specs=[any_spec] * 7,
        out_specs=pl.BlockSpec(memory_space=pltpu.VMEM),
        scratch_shapes=[
            pltpu.VMEM(A_k_cache.shape, bf16),
            pltpu.VMEM(A_v_cache.shape, bf16),
            pltpu.VMEM((A_wq.shape[0] // 2, A_wq.shape[1]), u32),
            pltpu.VMEM((A_wo.shape[0] // 2, A_wo.shape[1]), u32),
            pltpu.VMEM((B_w1.shape[0] // 2, B_w1.shape[1]), u32),
            pltpu.VMEM((B_w2.shape[0] // 2, B_w2.shape[1]), u32),
            pltpu.VMEM((B, D), A_x.dtype),
            pltpu.VMEM((Hkv, _R, _T), f32),
            pltpu.VMEM((2, NT, _R, _T), f32),
            pltpu.VMEM((2, NT, _R, _T), f32),
            pltpu.SemaphoreType.DMA((_AHEAD,)),
            pltpu.SemaphoreType.DMA((_AHEAD,)),
            pltpu.SemaphoreType.DMA((2,)),
        ],
        compiler_params=pltpu.CompilerParams(vmem_limit_bytes=100 * 1024 * 1024),
    )(A_x.reshape(B * Sq, D), A_k_cache, A_v_cache, A_wq, A_wo, B_w1, B_w2)
    return out.reshape(B, Sq, D)
```

```python
import jax
import jax.numpy as jnp
import jax.experimental.pallas as pl
import jax.experimental.pallas.tpu as pltpu

_T = 128
_R = 8
_CH = 2048
_AHEAD = 3
_TAIL = 1024


def _center(x):
    c = x - jnp.mean(x, axis=-1, keepdims=True)
    r = 1.0 / jnp.sqrt(jnp.mean(c * c, axis=-1, keepdims=True) + 1e-5)
    return c, r


@jax.jit
def pallas_interleave_layers__gqa_block_cached__dense_activation_silu__decode_kernel(
    A_x: jax.Array,
    A_k_cache: jax.Array,
    A_v_cache: jax.Array,
    A_wq: jax.Array,
    A_wo: jax.Array,
    B_x: jax.Array,
    B_w1: jax.Array,
    B_w2: jax.Array,
):
    del B_x
    B, Sq, D = A_x.shape
    _, Hkv, Sk, Dh = A_k_cache.shape
    HD = A_wq.shape[1]
    Hq = HD // Dh
    F = B_w1.shape[1]
    rep = Hq // Hkv
    assert Sq == 1 and Dh == _T and _R % rep == 0 and Hq % _R == 0 and B <= _R
    per = _R // rep
    NT = Sk // _T
    scale = float(Dh) ** -0.5
    f32, bf16 = jnp.float32, jnp.bfloat16

    def mm(a, b):
        return jnp.dot(a, b, preferred_element_type=f32)

    def kernel(x_hbm, k_hbm, v_hbm, wq_hbm, wo_hbm, w1_hbm, w2_hbm, ob,
               kb, vb, wqb, wob, w1b, w2b, xb, a_scr, s_scr, p_scr,
               ksem, vsem, wsem):
        def rows(src, dst, sem, b, h, lo, hi):
            r = pl.ds(lo, hi - lo)
            return pltpu.make_async_copy(src.at[b, h, r], dst.at[b, h, r], sem)

        def k_rows(n, lo, hi):
            return rows(k_hbm, kb, ksem.at[n % _AHEAD], n // Hkv, n % Hkv, lo, hi)

        def v_rows(n, lo, hi, sem=None):
            sem = vsem.at[n % _AHEAD] if sem is None else sem
            return rows(v_hbm, vb, sem, n // Hkv, n % Hkv, lo, hi)

        def start_rows(fn, n, lo, hi, step, **kw):
            for r in range(lo, hi, step):
                fn(n, r, min(r + step, hi), **kw).start()

        x_cp = pltpu.make_async_copy(x_hbm, xb, wsem.at[0])
        wq_cp, wo_cp, w1_cp, w2_cp = [
            pltpu.make_async_copy(s, d, wsem.at[i]) for s, d, i in
            ((wq_hbm, wqb, 0), (wo_hbm, wob, 1), (w1_hbm, w1b, 0), (w2_hbm, w2b, 0))]
        last = B * Hkv - 1
        cuts = (Sk - 2 * _TAIL, Sk - _TAIL, Sk)

        x_cp.start()
        wq_cp.start()

        row = jax.lax.broadcasted_iota(jnp.int32, (_R, _T), 0)
        zeros = jnp.zeros((_R, _T), f32)

        def tile(j):
            return pl.ds(pl.multiple_of(j * _T, _T), _T)

        def ld(w, b, h, j):
            return w[b, h, tile(j), :]

        def wt(w, i, j):
            return w[tile(i), tile(j)]

        def split(x):
            return [x[:, i * _T:(i + 1) * _T].astype(bf16) for i in range(x.shape[1] // _T)]

        def col(xs, w, j):
            y = None
            for i, xi in enumerate(xs):
                t = mm(xi, wt(w, i, j))
                y = t if y is None else y + t
            return y

        def q_head(xs, r, h):
            q = zeros
            for i in range(rep):
                q = jnp.where(row == (h % per) * rep + i, col(xs, wqb, h * rep + i), q)
            return (q * r).astype(bf16)

        def o_head(acc, a, h):
            for r in range(rep):
                ar = jnp.where(row == (h % per) * rep + r, a, 0.0).astype(bf16)
                acc = tuple(c + mm(ar, wt(wob, h * rep + r, j)) for j, c in enumerate(acc))
            return acc

        def fold(acc):
            acc = jnp.concatenate(acc, axis=1)
            return jnp.broadcast_to(jnp.sum(acc, axis=0, keepdims=True), (_R, D))

        def ffn(x):
            c, r = _center(x)
            xn = split(c)
            hs = []
            for j in range(F // _T):
                hid = col(xn, w1b, j) * r
                hs.append((hid * jax.nn.sigmoid(hid)).astype(bf16))
            return x + jnp.concatenate([col(hs, w2b, j) for j in range(D // _T)], axis=1)

        def first_pass_head(b, xs, r, h, acc):
            n = b * Hkv + h
            q = q_head(xs, r, h)
            k_rows(n, 0, Sk).wait()

            @pl.when(n + _AHEAD == Hkv)
            def _():
                w1_cp.start()
                w2_cp.start()

            @pl.when(n + _AHEAD <= last)
            def _():
                start_rows(k_rows, n + _AHEAD, 0, Sk, _CH)

            m = None
            for j in range(NT):
                kt = ld(kb, b, h, j).T
                kb[b, h, tile(j), :] = kt
                s = mm(q, kt) * scale
                s_scr[0, j] = s
                m = s if m is None else jnp.maximum(m, s)
            m = jnp.max(m, axis=-1, keepdims=True)
            l = zeros
            for j in range(NT):
                p = jnp.exp(s_scr[0, j] - m)
                l = l + p
                p_scr[0, j] = p
            inv = 1.0 / jnp.sum(l, axis=-1, keepdims=True)

            @pl.when(n == 0)
            def _():
                wo_cp.wait()

            @pl.when(n < last)
            def _():
                v_rows(n, 0, Sk).wait()

            @pl.when(n == last)
            def _():
                v_rows(n, 0, cuts[0]).wait()

            @pl.when(n + _AHEAD < last)
            def _():
                start_rows(v_rows, n + _AHEAD, 0, Sk, _CH)

            @pl.when(n + _AHEAD == last)
            def _():
                start_rows(v_rows, last, 0, cuts[0] - _CH, _CH)
                start_rows(v_rows, last, cuts[0] - _CH, cuts[0], _CH // 2)
                for i in range(2):
                    start_rows(v_rows, last, cuts[i], cuts[i + 1], _TAIL // 2, sem=wsem.at[i])

            o = zeros
            for i, (lo, hi) in enumerate(zip((0,) + cuts, cuts)):
                if i:
                    @pl.when(n == last)
                    def _():
                        v_rows(n, lo, hi, sem=wsem.at[i - 1]).wait()
                for j in range(lo // _T, hi // _T):
                    o = o + mm(p_scr[0, j].astype(bf16), ld(vb, b, h, j))
            return o_head(acc, o * inv, h)

        def qk_tile(b, h, q, slot, j, m):
            s = mm(q, ld(kb, b, h, j)) * scale
            s_scr[slot, j] = s
            return s if m is None else jnp.maximum(m, s)

        def exp_tile(slot, j, m, l):
            p = jnp.exp(s_scr[slot, j] - m)
            p_scr[slot, j] = p
            return l + p

        def pv_all(b, h):
            o = zeros
            for j in range(NT):
                o = o + mm(p_scr[h % 2, j].astype(bf16), ld(vb, b, h, j))
            return o

        def rowmax(m):
            return jnp.broadcast_to(jnp.max(m, axis=-1, keepdims=True), (_R, _T))

        def second_pass_step(b, h, m, q):
            mn, l, o = None, zeros, zeros
            for j in range(NT):
                mn = qk_tile(b, h + 1, q, (h + 1) % 2, j, mn)
                l = exp_tile(h % 2, j, m, l)
            o = pv_all(b, h)
            a_scr[h] = o / jnp.sum(l, axis=-1, keepdims=True)
            return rowmax(mn)

        def first_pass(b, x):
            c, r = _center(x)
            xs = split(c)
            return jax.lax.fori_loop(0, Hkv, lambda h, a: first_pass_head(b, xs, r, h, a),
                                     (zeros,) * (D // _T))

        def second_pass(b, x):
            c, r = _center(x)
            xs = split(c)
            qs = [q_head(xs, r, h) for h in range(Hkv)]
            m = None
            for j in range(NT):
                m = qk_tile(b, 0, qs[0], 0, j, m)
            m = rowmax(m)
            for h in range(Hkv - 2):
                m = second_pass_step(b, h, m, qs[h + 1])
            h = Hkv - 2
            mn, l = None, zeros
            for j in range(NT):
                mn = qk_tile(b, h + 1, qs[h + 1], (h + 1) % 2, j, mn)
                l = exp_tile(h % 2, j, m, l)
            m = rowmax(mn)
            l2, o = zeros, zeros
            for j in range(NT):
                o = o + mm(p_scr[h % 2, j].astype(bf16), ld(vb, b, h, j))
                l2 = exp_tile((h + 1) % 2, j, m, l2)
            a_scr[h] = o / jnp.sum(l, axis=-1, keepdims=True)
            o = pv_all(b, h + 1)
            acc = (zeros,) * (D // _T)
            for hh in range(Hkv - 1):
                acc = o_head(acc, a_scr[hh], hh)
            return o_head(acc, o / jnp.sum(l2, axis=-1, keepdims=True), h + 1)

        def layer_pair(i, x):
            b = i // 2
            first = i % 2 == 0

            @pl.when(i == 0)
            def _():
                wo_cp.start()
                x_cp.wait()
                wq_cp.wait()
                for n in range(_AHEAD):
                    start_rows(k_rows, n, 0, Sk, _CH)
                    start_rows(v_rows, n, 0, Sk, _CH)

            xin = xb[...].astype(f32)
            x0 = jnp.broadcast_to(xin[0:1], (_R, D))
            for bb in range(1, B):
                x0 = jnp.where(b == bb, jnp.broadcast_to(xin[bb:bb + 1], (_R, D)), x0)
            x = jnp.where(first, x0, x)

            acc = jax.lax.cond(first, lambda: first_pass(b, x), lambda: second_pass(b, x))

            @pl.when(i == 0)
            def _():
                w1_cp.wait()
                w2_cp.wait()

            x = ffn(x + fold(acc))
            ob[b] = x[0:1].astype(ob.dtype)
            return x

        jax.lax.fori_loop(0, 2 * B, layer_pair, jnp.zeros((_R, D), f32))

    any_spec = pl.BlockSpec(memory_space=pl.ANY)
    out = pl.pallas_call(
        kernel,
        out_shape=jax.ShapeDtypeStruct((B, Sq, D), A_x.dtype),
        in_specs=[any_spec] * 7,
        out_specs=pl.BlockSpec(memory_space=pltpu.VMEM),
        scratch_shapes=[
            pltpu.VMEM(A_k_cache.shape, bf16),
            pltpu.VMEM(A_v_cache.shape, bf16),
            pltpu.VMEM(A_wq.shape, bf16),
            pltpu.VMEM(A_wo.shape, bf16),
            pltpu.VMEM(B_w1.shape, bf16),
            pltpu.VMEM(B_w2.shape, bf16),
            pltpu.VMEM((B, D), A_x.dtype),
            pltpu.VMEM((Hkv, _R, _T), f32),
            pltpu.VMEM((2, NT, _R, _T), f32),
            pltpu.VMEM((2, NT, _R, _T), f32),
            pltpu.SemaphoreType.DMA((_AHEAD,)),
            pltpu.SemaphoreType.DMA((_AHEAD,)),
            pltpu.SemaphoreType.DMA((2,)),
        ],
        compiler_params=pltpu.CompilerParams(vmem_limit_bytes=100 * 1024 * 1024),
    )(A_x.reshape(B * Sq, D), A_k_cache, A_v_cache, A_wq, A_wo, B_w1, B_w2)
    return out.reshape(B, Sq, D)
```

```python
import jax
import jax.numpy as jnp
import jax.experimental.pallas as pl
import jax.experimental.pallas.tpu as pltpu

_T = 128
_R = 8
_CH = 2048
_AHEAD = 3
_RING = _AHEAD + 1
_QM = 5
_TAIL = 1024


def _center(x):
    c = x - jnp.mean(x, axis=-1, keepdims=True)
    r = 1.0 / jnp.sqrt(jnp.mean(c * c, axis=-1, keepdims=True) + 1e-5)
    return c, r


@jax.jit
def pallas_interleave_layers__gqa_block_cached__dense_activation_silu__decode_kernel(
    A_x: jax.Array,
    A_k_cache: jax.Array,
    A_v_cache: jax.Array,
    A_wq: jax.Array,
    A_wo: jax.Array,
    B_x: jax.Array,
    B_w1: jax.Array,
    B_w2: jax.Array,
):
    del B_x
    B, Sq, D = A_x.shape
    _, Hkv, Sk, Dh = A_k_cache.shape
    HD = A_wq.shape[1]
    Hq = HD // Dh
    F = B_w1.shape[1]
    rep = Hq // Hkv
    assert Sq == 1 and Dh == _T and _R % rep == 0 and Hq % _R == 0 and B <= _R
    per = _R // rep
    NT = Sk // _T
    scale = float(Dh) ** -0.5
    f32, bf16, u32 = jnp.float32, jnp.bfloat16, jnp.uint32

    def mm(a, b):
        return jnp.dot(a, b, preferred_element_type=f32)

    def kernel(x_hbm, k_hbm, v_hbm, wq_hbm, wo_hbm, w1_hbm, w2_hbm, ob,
               kb, vb, wqb, wob, w1b, w2b, xb, kp, vp, wqp, wop, w1p, w2p, wqf, wof, s_scr, p_scr,
               ksem, vsem, wsem):
        def rows(src, dst, sem, n, lo, hi):
            r = pl.ds(lo, hi - lo)
            return pltpu.make_async_copy(src.at[n // Hkv, n % Hkv, r], dst.at[n % _RING, r], sem)

        def k_rows(n, lo, hi):
            return rows(k_hbm, kb, ksem.at[n % _AHEAD], n, lo, hi)

        def v_rows(n, lo, hi, sem=None):
            return rows(v_hbm, vb, vsem.at[n % _AHEAD] if sem is None else sem, n, lo, hi)

        def start_rows(fn, n, lo, hi, step, **kw):
            for r in range(lo, hi, step):
                fn(n, r, min(r + step, hi), **kw).start()

        x_cp = pltpu.make_async_copy(x_hbm, xb, wsem.at[0])
        wq_cp, wo_cp, w1_cp, w2_cp = [
            pltpu.make_async_copy(s, d, wsem.at[i]) for s, d, i in
            ((wq_hbm, wqb, 0), (wo_hbm, wob, 1), (w1_hbm, w1b, 0), (w2_hbm, w2b, 0))]
        last = B * Hkv - 1
        cuts = (Sk - 2 * _TAIL, Sk - _TAIL, Sk)

        x_cp.start()
        wq_cp.start()

        row = jax.lax.broadcasted_iota(jnp.int32, (_R, _T), 0)
        zeros = jnp.zeros((_R, _T), f32)

        def tile(j):
            return pl.ds(pl.multiple_of(j * _T, _T), _T)

        def half(j):
            return pl.ds(pl.multiple_of(j * (_T // 2), _T // 2), _T // 2)

        def ld(w, h, j):
            return pltpu.bitcast(w[h, half(j), :], bf16)

        def wt(w, i, j):
            return pltpu.bitcast(w[half(i), tile(j)], bf16)

        def repack(src, packed, wide=None):
            def body(i, carry):
                w = src[tile(i), :]
                packed[half(i), :] = pltpu.bitcast(w, u32)
                if wide is not None:
                    wide[tile(i), :] = w.astype(f32)
                return carry
            jax.lax.fori_loop(0, src.shape[0] // _T, body, 0)

        def split(x):
            return [x[:, i * _T:(i + 1) * _T].astype(bf16) for i in range(x.shape[1] // _T)]

        def col(xs, w, j):
            y = None
            for i, xi in enumerate(xs):
                t = mm(xi, wt(w, i, j))
                y = t if y is None else y + t
            return y

        def q_head(xs, r, h):
            q = zeros
            for i in range(rep):
                q = jnp.where(row == (h % per) * rep + i, col(xs, wqp, h * rep + i), q)
            return (q * r).astype(bf16)

        def q_head_vpu(xt, r, h):
            q = zeros
            for i in range(rep):
                y = None
                for t, xi in enumerate(xt):
                    z = (xi * wqf[tile(t), tile(h * rep + i)]).reshape(_T // _R, _R, _T).sum(0)
                    y = z if y is None else y + z
                q = jnp.where(row == (h % per) * rep + i, jnp.sum(y, axis=0, keepdims=True), q)
            return (q * r).astype(bf16)

        def o_head(acc, a, h):
            for r in range(rep):
                ar = jnp.where(row == (h % per) * rep + r, a, 0.0).astype(bf16)
                acc = tuple(c + mm(ar, wt(wop, h * rep + r, j)) for j, c in enumerate(acc))
            return acc

        def o_row_vpu(acc, a, h, r, after=None):
            k = (h % per) * rep + r
            if after is not None:
                a = jnp.where(after[0], after[1], a)
            at = jnp.broadcast_to(a[k:k + 1], (_T, _T)).T
            return tuple(
                c + (at * wof[tile(h * rep + r), tile(j)]).reshape(_T // _R, _R, _T).sum(0)
                for j, c in enumerate(acc))

        def fold(acc):
            acc = jnp.concatenate(acc, axis=1)
            return jnp.broadcast_to(jnp.sum(acc, axis=0, keepdims=True), (_R, D))

        def ffn(x):
            c, r = _center(x)
            xn = split(c)
            hs = []
            for j in range(F // _T):
                hid = col(xn, w1p, j) * r
                hs.append((hid * jax.nn.sigmoid(hid)).astype(bf16))
            return x + jnp.concatenate([col(hs, w2p, j) for j in range(D // _T)], axis=1)

        def first_pass_head(b, xs, r, h, acc):
            n = b * Hkv + h
            q = q_head(xs, r, h)
            k_rows(n, 0, Sk).wait()

            @pl.when(n + _AHEAD == Hkv)
            def _():
                w1_cp.start()
                w2_cp.start()

            @pl.when(n + _AHEAD <= last)
            def _():
                start_rows(k_rows, n + _AHEAD, 0, Sk, _CH)

            m = None
            for j in range(NT):
                kt = kb[n % _RING, tile(j), :].T
                kp[h, half(j), :] = pltpu.bitcast(kt, u32)
                s = mm(q, kt) * scale
                s_scr[0, j] = s
                m = s if m is None else jnp.maximum(m, s)
            m = jnp.max(m, axis=-1, keepdims=True)
            l = zeros
            for j in range(NT):
                p = jnp.exp(s_scr[0, j] - m)
                l = l + p
                p_scr[0, j] = p
            inv = 1.0 / jnp.sum(l, axis=-1, keepdims=True)

            @pl.when(n == 0)
            def _():
                wo_cp.wait()
                repack(wob, wop, wof)

            @pl.when(n < last)
            def _():
                v_rows(n, 0, Sk).wait()

            @pl.when(n == last)
            def _():
                v_rows(n, 0, cuts[0]).wait()

            @pl.when(n + _AHEAD < last)
            def _():
                start_rows(v_rows, n + _AHEAD, 0, Sk, _CH)

            @pl.when(n + _AHEAD == last)
            def _():
                start_rows(v_rows, last, 0, cuts[0] - _CH, _CH)
                start_rows(v_rows, last, cuts[0] - _CH, cuts[0], _CH // 2)
                for i in range(2):
                    start_rows(v_rows, last, cuts[i], cuts[i + 1], _TAIL // 2, sem=wsem.at[i])

            o = zeros
            for i, (lo, hi) in enumerate(zip((0,) + cuts, cuts)):
                if i:
                    @pl.when(n == last)
                    def _():
                        v_rows(n, lo, hi, sem=wsem.at[i - 1]).wait()
                for j in range(lo // _T, hi // _T):
                    v = vb[n % _RING, tile(j), :]
                    vp[h, half(j), :] = pltpu.bitcast(v, u32)
                    o = o + mm(p_scr[0, j].astype(bf16), v)
            return o_head(acc, o * inv, h)

        def qk_tile(b, h, q, slot, j, m):
            s = mm(q, ld(kp, h, j)) * scale
            s_scr[slot, j] = s
            return s if m is None else jnp.maximum(m, s)

        def exp_tile(slot, j, m, l):
            p = jnp.exp(s_scr[slot, j] - m)
            p_scr[slot, j] = p
            return l + p

        def pv_all(b, h):
            o = zeros
            for j in range(NT):
                o = o + mm(p_scr[h % 2, j].astype(bf16), ld(vp, h, j))
            return o

        def rowmax(m):
            return jnp.broadcast_to(jnp.max(m, axis=-1, keepdims=True), (_R, _T))

        def first_pass(b, x):
            c, r = _center(x)
            xs = split(c)
            return jax.lax.fori_loop(0, Hkv, lambda h, a: first_pass_head(b, xs, r, h, a),
                                     (zeros,) * (D // _T))

        def second_pass(b, x):
            c, r = _center(x)
            xs = split(c)
            xt = [jnp.broadcast_to(c[0:1, t * _T:(t + 1) * _T], (_T, _T)).T for t in range(D // _T)]
            qs = [q_head(xs, r, h) if h < _QM else q_head_vpu(xt, r, h) for h in range(Hkv)]
            m = None
            for j in range(NT):
                m = qk_tile(b, 0, qs[0], 0, j, m)
            m = rowmax(m)
            acc = (zeros,) * (D // _T)
            never = row == _R + b
            gap = NT // rep
            a = None
            for h in range(Hkv - 1):
                mn, l = None, zeros
                for j in range(NT):
                    mn = qk_tile(b, h + 1, qs[h + 1], (h + 1) % 2, j, mn)
                    l = exp_tile(h % 2, j, m, l)
                    if a is not None and j % gap == 0:
                        acc = o_row_vpu(acc, a, h - 1, j // gap, (never, mn))
                m = rowmax(mn)
                l2, o = zeros, zeros
                for j in range(NT):
                    o = o + mm(p_scr[h % 2, j].astype(bf16), ld(vp, h, j))
                    if h + 2 == Hkv:
                        l2 = exp_tile((h + 1) % 2, j, m, l2)
                a = o / jnp.sum(l, axis=-1, keepdims=True)
            h, o = Hkv - 1, zeros
            for j in range(NT):
                o = o + mm(p_scr[h % 2, j].astype(bf16), ld(vp, h, j))
                if j % gap == 0:
                    acc = o_row_vpu(acc, a, h - 1, j // gap, (never, o))
            return o_head(acc, o / jnp.sum(l2, axis=-1, keepdims=True), h)

        def layer_pair(i, x):
            b = i // 2
            first = i % 2 == 0

            @pl.when(i == 0)
            def _():
                wo_cp.start()
                x_cp.wait()
                wq_cp.wait()
                for n in range(_AHEAD):
                    start_rows(k_rows, n, 0, Sk, _CH)
                    start_rows(v_rows, n, 0, Sk, _CH)
                repack(wqb, wqp, wqf)

            xin = xb[...].astype(f32)
            x0 = jnp.broadcast_to(xin[0:1], (_R, D))
            for bb in range(1, B):
                x0 = jnp.where(b == bb, jnp.broadcast_to(xin[bb:bb + 1], (_R, D)), x0)
            x = jnp.where(first, x0, x)

            acc = jax.lax.cond(first, lambda: first_pass(b, x), lambda: second_pass(b, x))

            @pl.when(i == 0)
            def _():
                w1_cp.wait()
                w2_cp.wait()
                repack(w1b, w1p)
                repack(w2b, w2p)

            x = ffn(x + fold(acc))
            ob[b] = x[0:1].astype(ob.dtype)
            return x

        jax.lax.fori_loop(0, 2 * B, layer_pair, jnp.zeros((_R, D), f32))

    any_spec = pl.BlockSpec(memory_space=pl.ANY)
    out = pl.pallas_call(
        kernel,
        out_shape=jax.ShapeDtypeStruct((B, Sq, D), A_x.dtype),
        in_specs=[any_spec] * 7,
        out_specs=pl.BlockSpec(memory_space=pltpu.VMEM),
        scratch_shapes=[
            pltpu.VMEM((_RING, Sk, Dh), bf16),
            pltpu.VMEM((_RING, Sk, Dh), bf16),
            pltpu.VMEM(A_wq.shape, bf16),
            pltpu.VMEM(A_wo.shape, bf16),
            pltpu.VMEM(B_w1.shape, bf16),
            pltpu.VMEM(B_w2.shape, bf16),
            pltpu.VMEM((B, D), A_x.dtype),
            pltpu.VMEM((Hkv, Sk // 2, Dh), u32),
            pltpu.VMEM((Hkv, Sk // 2, Dh), u32),
            *[pltpu.VMEM((w.shape[0] // 2, w.shape[1]), u32) for w in (A_wq, A_wo, B_w1, B_w2)],
            pltpu.VMEM(A_wq.shape, f32),
            pltpu.VMEM(A_wo.shape, f32),
            pltpu.VMEM((2, NT, _R, _T), f32),
            pltpu.VMEM((2, NT, _R, _T), f32),
            pltpu.SemaphoreType.DMA((_AHEAD,)),
            pltpu.SemaphoreType.DMA((_AHEAD,)),
            pltpu.SemaphoreType.DMA((2,)),
        ],
        compiler_params=pltpu.CompilerParams(vmem_limit_bytes=100 * 1024 * 1024),
    )(A_x.reshape(B * Sq, D), A_k_cache, A_v_cache, A_wq, A_wo, B_w1, B_w2)
    return out.reshape(B, Sq, D)
```
